```python
import os as _os
_os.environ.setdefault("JAX_PLATFORMS", "cpu")
import jax
import jax.numpy as jnp

def _softmax(x, axis=-1):
    return jax.nn.softmax(x, axis=axis)
def _gelu(x):
    return jax.nn.gelu(x, approximate=True)
def _silu(x):
    return jax.nn.silu(x)
def _sigmoid(x):
    return jax.nn.sigmoid(x)
def _layernorm(x, axis=-1, eps=1e-5):
    m = jnp.mean(x, axis=axis, keepdims=True)
    v = jnp.var(x, axis=axis, keepdims=True)
    return (x - m) / jnp.sqrt(v + eps)
def _scatter_add(tgt, idx, src, axis=0):
    return tgt.at[idx].add(src)
def _segment_sum(src, seg, n):
    return jax.ops.segment_sum(src, seg, n)
class _Rng:
    def __init__(self, key):
        self._k = key
    def _next(self):
        self._k, sub = jax.random.split(self._k)
        return sub
    def normal(self, shape):
        return jax.random.normal(self._next(), shape, dtype=jnp.bfloat16)
    def randint(self, lo, hi, shape):
        return jax.random.randint(self._next(), shape, lo, hi, dtype=jnp.int32)
    def uniform(self, shape, lo=0.0, hi=1.0):
        return jax.random.uniform(self._next(), shape, jnp.bfloat16, lo, hi)
    def permutation(self, n):
        return jax.random.permutation(self._next(), n)


kernel_name = 'concat_heads__mha_block_cached__mha_block_cached__near_ridge'

def setup_inputs():
    _rng = _Rng(jax.random.key(int.from_bytes(__import__("os").urandom(4), "little")))
    _w = (lambda a: (lambda t: t.astype(jnp.bfloat16) if jnp.issubdtype(t.dtype, jnp.floating) else t)(jnp.asarray(a)))
    def _A_setup():
        B, Sq, D = 16, 32, 1024
        H, Sk, Dh = 32, 32, 128
        return {
            "x": _w((lambda *s: _rng.normal(s) * 0.8)(B, Sq, D)),
            "k_cache": _w((lambda *s: _rng.normal(s) * 0.8)(B, H, Sk, Dh)),
            "v_cache": _w((lambda *s: _rng.normal(s) * 0.05)(B, H, Sk, Dh)),
            "wq": _w((lambda *s: _rng.normal(s) * 0.8)(D, H * Dh) * (D ** -0.5)),
            "wo": _w((lambda *s: _rng.normal(s) * 0.05)(H * Dh, D) * ((H * Dh) ** -0.5)),
        }
    _A_in = _A_setup()

    def _B_setup():
        B, Sq, D = 16, 32, 1024
        H, Sk, Dh = 32, 32, 128
        return {
            "x": _w((lambda *s: _rng.normal(s) * 0.8)(B, Sq, D)),
            "k_cache": _w((lambda *s: _rng.normal(s) * 0.8)(B, H, Sk, Dh)),
            "v_cache": _w((lambda *s: _rng.normal(s) * 0.05)(B, H, Sk, Dh)),
            "wq": _w((lambda *s: _rng.normal(s) * 0.8)(D, H * Dh) * (D ** -0.5)),
            "wo": _w((lambda *s: _rng.normal(s) * 0.05)(H * Dh, D) * ((H * Dh) ** -0.5)),
        }
    _B_in = _B_setup()

    return {
        "A_x": _A_in["x"],
        "A_k_cache": _A_in["k_cache"],
        "A_v_cache": _A_in["v_cache"],
        "A_wq": _A_in["wq"],
        "A_wo": _A_in["wo"],
        "B_x": _B_in["x"],
        "B_k_cache": _B_in["k_cache"],
        "B_v_cache": _B_in["v_cache"],
        "B_wq": _B_in["wq"],
        "B_wo": _B_in["wo"],
    }

def reference(A_x, A_k_cache, A_v_cache, A_wq, A_wo, B_x, B_k_cache, B_v_cache, B_wq, B_wo):
    def _A_ref(x, k_cache, v_cache, wq, wo):
        B, Sq, D = x.shape
        H, Dh = 32, 128
        q = (lambda x, *d: x.transpose(*d))((x @ wq).reshape(B, Sq, H, Dh), 0, 2, 1, 3)
        scores = jnp.einsum("bhqd,bhkd->bhqk", q, k_cache) * (Dh ** -0.5)
        p = _softmax(scores, axis=-1)
        o = jnp.einsum("bhqk,bhkd->bhqd", p, v_cache)
        return (lambda x, *d: x.transpose(*d))(o, 0, 2, 1, 3).reshape(B, Sq, H * Dh) @ wo

    def _B_ref(x, k_cache, v_cache, wq, wo):
        B, Sq, D = x.shape
        H, Dh = 32, 128
        q = (lambda x, *d: x.transpose(*d))((x @ wq).reshape(B, Sq, H, Dh), 0, 2, 1, 3)
        scores = jnp.einsum("bhqd,bhkd->bhqk", q, k_cache) * (Dh ** -0.5)
        p = _softmax(scores, axis=-1)
        o = jnp.einsum("bhqk,bhkd->bhqd", p, v_cache)
        return (lambda x, *d: x.transpose(*d))(o, 0, 2, 1, 3).reshape(B, Sq, H * Dh) @ wo

    a = _A_ref(A_x, A_k_cache, A_v_cache, A_wq, A_wo)
    b = _B_ref(B_x, B_k_cache, B_v_cache, B_wq, B_wo)
    return jnp.concatenate([a, b], axis=-1)
```

```python
import functools, contextlib, itertools
import numpy as np
import jax
import jax.numpy as jnp
from jax import lax
import jax.experimental.pallas as pl
import jax.experimental.pallas.tpu as pltpu

B, SQ, D = 16, 32, 1024
H, SK, DH = 32, 32, 128
M = B * SQ
GB = 128 // SK
G = 8
NG = H // G
NS = 2 * NG
BM, BK = M // 4, D // 4
F32, BF16, U32 = jnp.float32, jnp.bfloat16, jnp.uint32

LHS = (((1, 0, 0), (1, 1, 1)), ((1, 1, 0), (1, 1, 1)), ((1, 0, 0), (1, 0, 1)), ((1, 1, 1),),
       ((1, 0, 1), (-1, 1, 1)), ((1, 0, 0),), ((1, 1, 0), (-1, 0, 0)))
RHS = (((1, 0, 0), (1, 1, 1)), ((1, 0, 0),), ((1, 1, 1),), ((1, 1, 0), (-1, 0, 0)),
       ((1, 1, 0), (1, 1, 1)), ((1, 0, 1), (-1, 1, 1)), ((1, 0, 0), (1, 0, 1)))
OUT = {(0, 0): ((1, 0), (-1, 2), (1, 3), (1, 4)), (0, 1): ((1, 2), (1, 5)),
       (1, 0): ((1, 1), (1, 3)), (1, 1): ((1, 0), (-1, 1), (1, 5), (1, 6))}


def _term(spec, x):
    v = x(*spec[0][1:])
    for sign, *idx in spec[1:]:
        v = v + x(*idx) if sign > 0 else v - x(*idx)
    return v


def _outer(spec, blk):
    return lambda r, c: _term(spec, lambda i, j: blk(2 * i + r, 2 * j + c))


class _Combiner:
    def __init__(self):
        self.m, self.done = {}, set()

    def add(self, i, val):
        self.m[i] = val

    def ready(self):
        order = list(self.m)
        for rc, spec in OUT.items():
            if rc not in self.done and all(i in self.m for _, i in spec):
                self.done.add(rc)
                spec = sorted(spec, key=lambda t: order.index(t[1]))
                if spec[0][0] < 0:
                    spec[0], spec[1] = spec[1], spec[0]
                yield rc, _term(spec, lambda i: self.m[i])


def _mm(a, b):
    return jnp.dot(a, b, preferred_element_type=F32)


def _ld(ref, idx):
    return pltpu.bitcast(ref.bitcast(U32)[idx], BF16)


def _kernel(ax, ak, av, awq, awo, bx, bk, bv, bwq, bwo, out_hbm,
            x_buf, xb_buf, xs_buf, wq_buf, k_buf, v_buf, wo_buf, acc, out_buf, q_buf, fence_ref, sems, osem,
            *, cfg):
    srcs = ((ax, ak, av, awq, awo), (bx, bk, bv, bwq, bwo))
    nodma, porder = cfg["nodma"], cfg["porder"]
    scope = jax.named_scope if cfg["prof"] else (lambda n: contextlib.nullcontext())

    def wait(buf, sem):
        if nodma: return
        pltpu.make_async_copy(buf, buf, sem).wait()

    def fence():
        fence_ref[0] = 0

    def xq(r, c):
        idx = (pl.ds(r * M // 2, M // 2), pl.ds(c * D // 2, D // 2))
        return pltpu.make_async_copy(ax.at[idx], x_buf.at[idx], sems.at[5, 2 * r + c])

    def wq0(r, c):
        idx = (pl.ds(r * D // 2, D // 2), pl.ds(c * D // 2, D // 2))
        return pltpu.make_async_copy(awq.at[idx], wq_buf.at[(0,) + idx], sems.at[5, 4 + 2 * r + c])

    def wq1(r, c):
        rows, cols = pl.ds(r * D // 2, D // 2), c * D // 2
        return pltpu.make_async_copy(awq.at[rows, pl.ds(D + cols, D // 2)], wq_buf.at[1, rows, pl.ds(cols, D // 2)],
                                     sems.at[4, 4 + 2 * r + c])

    def xb(half):
        rows = pl.ds(half * (BM // 2), BM // 2)
        return pltpu.make_async_copy(bx.at[:, rows], xb_buf.at[:, rows], sems.at[4, half])

    need, seen = [], set()
    for i1 in porder:
        cur = [("x", r, c) for _, r, c in LHS[i1]] + [("w", r, c) for _, r, c in RHS[i1]]
        need.append([t for t in cur if t not in seen])
        seen.update(cur)
    first_copy = lambda t: (xq if t[0] == "x" else wq0)(t[1], t[2])

    if not nodma:
        for grp in need:
            for t in grp:
                first_copy(t).start()
        for s in range(NS):
            br, g = divmod(s, NG)
            x, k, v, wq, wo = srcs[br]
            if s == 0:
                for rc in ((0, 0), (1, 1), (1, 0), (0, 1)):
                    wq1(*rc).start()
            elif s + 1 < NS:
                br1, g1 = divmod(s + 1, NG)
                pltpu.make_async_copy(srcs[br1][3].at[:, pl.ds(g1 * G * DH, G * DH)], wq_buf.at[s + 1], sems.at[0, s + 1]).start()
            pltpu.make_async_copy(k.at[:, pl.ds(g * G, G)], k_buf.at[s], sems.at[1, s]).start()
            pltpu.make_async_copy(v.at[:, pl.ds(g * G, G)], v_buf.at[s], sems.at[2, s]).start()
            pltpu.make_async_copy(wo.at[pl.ds(g * G * DH, G * DH), :], wo_buf.at[s], sems.at[3, s]).start()
            if s in (1, 2):
                xb(s - 1).start()

    scale = DH ** -0.5

    def lhs_terms(blk, i1):
        t = _outer(LHS[i1], blk)
        t = {(r, c): t(r, c) for r in range(2) for c in range(2)}
        return [_term(LHS[i2], lambda r, c: t[r, c]) for i2 in range(7)]

    def xprep(br, i1):
        for j in range(2):
            blk = lambda r, c: x_buf[r * BM:(r + 1) * BM, c * BK + j * 128:c * BK + (j + 1) * 128].astype(F32)
            for i2, val in enumerate(lhs_terms(blk, i1)):
                xs_buf[0, 7 * i1 + i2, j] = val.astype(BF16)

    def xpiece(s, n, anchor):
        nr = cfg["xstrip"]
        i1, rest = divmod(n, 2 * (BM // 2 // nr))
        j, k = divmod(rest, BM // 2 // nr)
        r0 = pl.multiple_of((s % 2) * (BM // 2) + k * nr, nr)
        blk = lambda r, c: xb_buf[r, pl.ds(r0, nr), c * BK + j * 128:c * BK + (j + 1) * 128].astype(F32)
        t = _outer(LHS[i1], blk)
        t = {(r, c): t(r, c) for r in range(2) for c in range(2)}
        for d in range(2):
            t[d, d] = jnp.where(s > 0, t[d, d], anchor[k * nr:(k + 1) * nr])
        for i2 in range(7):
            xs_buf[1, 7 * i1 + i2, j, pl.ds(r0, nr)] = _term(LHS[i2], lambda r, c: t[r, c]).astype(BF16)

    def products(lhs, w_ref, s, i1, inner_order):
        def t(r, c, j):
            blk = lambda rr, cc: w_ref[s, rr * BK:(rr + 1) * BK, cc * BK + j * 128:cc * BK + (j + 1) * 128].astype(F32)
            return _outer(RHS[i1], blk)(r, c)
        keep = {}
        def get(j):
            local = {}
            def f(r, c):
                store = keep if (r == c and len(RHS[i1]) > 1) else local
                if (r, c, j) not in store:
                    store[r, c, j] = t(r, c, j)
                return store[r, c, j]
            return f
        def prod(i2, j, f):
            return i2, j, _mm(lhs(i2), _term(RHS[i2], f).astype(BF16))
        for tok in inner_order:
            fence()
            if tok == "C":
                yield prod(0, 0, get(0)), prod(0, 1, get(1))
            else:
                i2, j = {"A": 1, "B": 3, "D": 5}[tok[0]], int(tok[1])
                f = get(j)
                yield prod(i2, j, f), prod(i2 + 1, j, f)

    def strassen(lhs_for, w_ref, s, emit, order, inner_order):
        outer = {(r, c, j): _Combiner() for r in range(2) for c in range(2) for j in range(2)}
        for i1 in order:
            inner = [_Combiner(), _Combiner()]
            for pair in products(lhs_for(i1), w_ref, s, i1, inner_order):
                for i2, j, val in pair:
                    inner[j].add(i2, val)
                for j in range(2):
                    for (r, c), val in inner[j].ready():
                        outer[r, c, j].add(i1, val)
                        for (R, C), res in outer[r, c, j].ready():
                            emit(2 * R + r, 2 * C + c, j, res)
                yield pair[0][2]

    def qproj(s, br, first, jit_x=False):
        def lhs_for(i1):
            if first:
                for t in need[porder.index(i1)]:
                    if not nodma: first_copy(t).wait()
            if jit_x:
                xprep(br, i1)
            return lambda i2: jnp.concatenate([_ld(xs_buf, (br, 7 * i1 + i2, j)) for j in range(2)], axis=1)
        def emit(r, c, j, val):
            q_buf[2 * c + j, r * BM:(r + 1) * BM] = val.astype(BF16)
        return strassen(lhs_for, wq_buf, s, emit, porder if first else cfg["qorder"], cfg["qinner"])

    def qk(s, items, qs):
        ps = []
        lane = lax.broadcasted_iota(jnp.int32, (SK, 128), 1) // SQ
        for gb, h in items:
            kk = pltpu.bitcast(k_buf.bitcast(U32)[s, gb * GB:(gb + 1) * GB, h].reshape(64, DH), BF16)
            st = lax.dot_general(kk, qs(gb, h), (((1,), (1,)), ((), ())), preferred_element_type=F32)
            sc = jnp.where(lane == 0, st[0:32], jnp.where(lane == 1, st[32:64], jnp.where(lane == 2, st[64:96], st[96:128])))
            sc = sc * scale
            m = jnp.max(sc, axis=0, keepdims=True)
            e = jnp.exp(sc - m)
            l = jnp.sum(e, axis=0, keepdims=True)
            pr = e * (1.0 / l)
            ps.append(jnp.concatenate([jnp.where(lane == j, pr, 0.0) for j in range(GB)], axis=0).astype(BF16))
        return ps

    def pv(s, items, ps, o):
        for (gb, h), p in zip(items, ps):
            vv = pltpu.bitcast(v_buf.bitcast(U32)[s, gb * GB:(gb + 1) * GB, h].reshape(64, DH), BF16)
            o[gb, h] = lax.dot_general(p, vv, (((0,), (0,)), ((), ())), preferred_element_type=F32)

    def att_items(n):
        quad, j = divmod(n, 2)
        R, C = ((1, 1), (0, 0), (1, 0), (0, 1))[quad]
        return [(2 * R + r, 2 * (2 * C + c) + j) for r in range(2) for c in range(2)]

    def oterms(o, terms, i1):
        if i1 not in terms:
            t = [lhs_terms(lambda r, c: o[r, 2 * c + j], i1) for j in range(2)]
            terms[i1] = [jnp.concatenate([a, b], axis=1).astype(BF16) for a, b in zip(*t)]
        return terms[i1]

    def oproj(s, o, terms, mode):
        def lhs_for(i1):
            t = oterms(o, terms, i1)
            return lambda i2: t[i2]
        done = set()
        def emit(r, c, j, val):
            idx = (2 * c + j, slice(r * BM, (r + 1) * BM))
            if mode != "F":
                val = val + acc[idx]
            if mode == "A":
                acc[idx] = jnp.where(s == NG - 1, 0.0, val)
                out_buf[(0,) + idx] = val.astype(BF16)
            elif mode == "E":
                out_buf[(1,) + idx] = val.astype(BF16)
                done.add((r, c, j))
                if (r ^ 1, c, j) in done:
                    rows = pl.ds(r // 2 * M // 2, M // 2)
                    pltpu.make_async_copy(out_buf.at[1, idx[0], rows], out_hbm.at[rows, pl.ds(D + idx[0] * 128, 128)],
                                          osem.at[1]).start()
            else:
                acc[idx] = val
        return strassen(lhs_for, wo_buf, s, emit, cfg["eorder"] if mode == "E" else cfg["oorder"], cfg["oinner"])

    def out_copies(br, R, C):
        rows = pl.ds(R * M // 2, M // 2)
        return [pltpu.make_async_copy(out_buf.at[br, n, rows], out_hbm.at[rows, pl.ds(br * D + n * 128, 128)], osem.at[br])
                for n in range(4 * C, 4 * C + 4)]

    def body(s, mode):
        ps, o, qv, terms = {}, {}, {}, {}
        xcount = itertools.count()
        def qs(gb, h):
            if (gb, h) not in qv:
                qv[gb, h] = _ld(q_buf, (h, slice(gb * 64, (gb + 1) * 64)))
            return qv[gb, h]
        qp = qproj(s, {"F": 0, "B": 1}.get(mode, s // NG), False) if mode != "E" else iter(())
        op = oproj(s - 1, o, terms, mode)
        for t in cfg["sched" + mode]:
            kind, n = t[0], (int(t[1:]) if t[1:].isdigit() else None)
            if kind == "Q":
                for _ in range(n):
                    anchor = next(qp)
            elif kind == "O":
                for _ in range(n):
                    anchor = next(op)
            elif kind == "L":
                for gb in range(4):
                    for h in range(G):
                        qs(gb, h)
            elif kind == "K":
                ps[n] = qk(s - 1, att_items(n), qs)
            elif kind == "V":
                pv(s - 1, att_items(n), ps.pop(n), o)
            elif kind == "T":
                for c in t[1:]:
                    oterms(o, terms, int(c))
            elif kind == "X":
                for _ in range(n):
                    xpiece(s, next(xcount), anchor)
            elif kind == "W":
                with scope("wait"):
                    for c in t[1:]:
                        if c in "ab":
                            for rc in (((0, 0), (1, 1)) if c == "a" else ((1, 0), (0, 1))):
                                if not nodma: wq1(*rc).wait()
                            continue
                        if c == "x":
                            if not nodma: pl.when(s < NG)(lambda: xb(s - 2).wait())
                            continue
                        i = s if c == "0" else s - 1
                        wait((wq_buf, k_buf, v_buf, wo_buf)[int(c)].at[i], sems.at[int(c), i])
            elif kind == "S":
                for c in t[1:]:
                    for cp in out_copies(1, int(c) // 2, int(c) % 2): cp.start()
        assert next(qp, None) is None and next(op, None) is None

    only = cfg["only"]
    if only in ("", "Q"):
        with scope("q0"):
            for _ in qproj(0, 0, True, True): pass
    if only in ("", "F"):
        with scope("bodyF"):
            body(1, "F")

    def step_a(s, _):
        with scope("bodyA"):
            body(s, "A")
        return 0

    def step_b(s, _):
        with scope("bodyB"):
            body(s, "B")
        return 0

    if only in ("", "A"):
        lax.fori_loop(2, NG + 1, step_a, 0)
        for n in range(8):
            pltpu.make_async_copy(out_buf.at[0, n], out_hbm.at[:, pl.ds(n * 128, 128)], osem.at[0]).start()
    if only in ("", "B"):
        lax.fori_loop(NG + 1, NS, step_b, 0)
    if only in ("", "E"):
        with scope("last"):
            body(NS, "E")
        pltpu.make_async_copy(out_buf.at[1], out_buf.at[1], osem.at[1]).wait()
    if only in ("", "A"):
        pltpu.make_async_copy(out_buf.at[0], out_buf.at[0], osem.at[0]).wait()


ATT1 = "K0 Q1 K1 Q1 V0 Q1 K2 Q1 V1 Q1 K3 Q1 V2 Q1 K4 Q1 V3 Q1 K5 Q1 V4 Q1 K6 Q1 V5 Q1 K7 Q1 V6 Q1 V7"
ATT0 = "K0 K1 Q1 V0 K2 Q1 V1 K3 Q1 V2 K4 Q1 V3 K5 Q1 V4 K6 Q1 V5 K7 Q1 V6 Q1 V7"
KS = "K0 Q1 K1 Q1 K2 Q1 K3 Q1 K4 Q1 K5 Q1 K6 Q1 K7"
VS = "V0 Q1 V1 Q1 V2 Q1 V3 Q1 V4 Q1 V5 Q1 V6 Q1 V7"
SCHED_F = {
    0: f"Wab Q20 L0 Q12 W12 {ATT1} T0123456 Q2 W3 O49",
    1: f"Wab Q20 L0 Q12 W12 {ATT0} T0123456 Q9 W3 O49",
    2: f"Wab Q20 L0 Q14 W12 {ATT1} T0123456 W3 O49",
    3: "Wa Q18 Wb1 K0 K1 Q1 K2 K3 Q1 K4 K5 Q1 K6 K7 Q8 W2 V0 Q1 V1 Q1 V2 Q1 V3 Q1 V4 Q1 V5 Q1 V6 Q1 V7 T0123456 Q13 W3 O49",
}
SCHED_A = {
    0: f"W01 Q1 {KS} Q27 W23x {VS} T0123456 Q7 O49",
    1: f"W012 Q1 {ATT1} T0123456 Q33 W3x O49",
    2: f"W01 Q1 {KS} Q33 W23x {VS} T0123456 Q1 O49",
    3: f"W01 Q13 {KS} Q15 W23x {VS} T0123456 Q7 O49",
    4: f"W01 Q1 {KS} Q30 W23x {VS} T0123456 Q4 O49",
    5: f"W01 Q13 {KS} Q18 W23x {VS} T0123456 Q4 O49",
}
SCHED_G = {0: ""}
SCHED_B = {
    0: f"W0123 Q1 {ATT1} Q33 O49",
    1: f"W0123 Q1 {ATT0} Q40 O49",
    2: f"W0123 {ATT1} Q34 O49",
    3: f"W0123 Q1 {ATT1} T0123456 Q33 O49",
}
SCHED_E = {
    0: "W123 K0 K1 K2 V0 K3 V1 K4 V2 K5 V3 K6 V4 K7 V5 V6 V7 O49",
    2: "W123 K0 K1 K2 V0 K3 V1 K4 V2 V3 O1 K5 O1 V4 O1 K6 O1 V5 O1 K7 O1 V6 O1 V7 O42",
    3: "W123 K0 K1 K2 V0 K3 V1 K4 V2 K5 V3 K6 O1 V4 O1 K7 O1 V5 O1 V6 O1 V7 O44",
    4: "W123 K0 K1 K2 K3 V0 V1 K4 V2 K5 V3 K6 O1 V4 O1 K7 O1 V5 O1 V6 O1 V7 O44",
    5: "W123 K0 K1 K2 V0 K3 V1 K4 O1 V2 O1 K5 O1 V3 O1 K6 O1 V4 O1 K7 O1 V5 O1 V6 O1 V7 O40",
}
INNER = {
    0: "C A0 B0 D0 A1 B1 D1",
    1: "A0 A1 C B0 D0 B1 D1",
    2: "A0 A1 C B0 B1 D0 D1",
    3: "A0 B0 A1 C D0 B1 D1",
    4: "A0 A1 B0 C D0 B1 D1",
    5: "A0 B0 A1 D0 C B1 D1",
    6: "A0 B0 A1 B1 C D0 D1",
    7: "A0 B0 D0 A1 C B1 D1",
}


def build(sf=3, sg=0, sa=0, sb=0, se=3, flags=None, nodma=False, only="", porder="1302456", qinner=5, oinner=5,
          qorder="0123456", oorder="0123456", eorder="0123456", prof=False, xb_at=2, xstrip=16, xunroll=1, pin=(2, 20)):
    digits = lambda v: [int(c) for c in str(v).zfill(7)]
    tok = lambda v, table: (table[v] if v in table else v.replace("_", " ")).split()
    if pin:
        lo, hi = pin
        n = 7 * 2 * (BM // 2 // xstrip)
        sp = " ".join(f"O1 X{(i + 1) * n // (hi - lo) - i * n // (hi - lo)}" for i in range(hi - lo))
        sa = (SCHED_A[sa].replace("O49", f"O{lo} {sp} O{49 - hi}")).replace(" ", "_")
    cfg = dict(pin=pin, schedG=tok(sg, SCHED_G), schedF=tok(sf, SCHED_F), schedA=tok(sa, SCHED_A), schedB=tok(sb, SCHED_B), schedE=tok(se, SCHED_E), nodma=nodma, only=only,
               porder=digits(porder), qorder=digits(qorder), oorder=digits(oorder), eorder=digits(eorder),
               qinner=tok(qinner, INNER), oinner=tok(oinner, INNER), prof=prof, xstrip=xstrip, xunroll=xunroll, xb_at=xb_at)

    def fn(A_x, A_k_cache, A_v_cache, A_wq, A_wo, B_x, B_k_cache, B_v_cache, B_wq, B_wo):
        out = pl.pallas_call(
            functools.partial(_kernel, cfg=cfg),
            out_shape=jax.ShapeDtypeStruct((M, 2 * D), BF16),
            in_specs=[pl.BlockSpec(memory_space=pl.ANY)] * 10,
            out_specs=pl.BlockSpec(memory_space=pl.ANY),
            scratch_shapes=[
                pltpu.VMEM((M, D), BF16),
                pltpu.VMEM((4, BM, D), BF16),
                pltpu.VMEM((2, 49, 2, BM, 128), BF16),
                pltpu.VMEM((NS, D, G * DH), BF16),
                pltpu.VMEM((NS, B, G, SK, DH), BF16),
                pltpu.VMEM((NS, B, G, SK, DH), BF16),
                pltpu.VMEM((NS, G * DH, D), BF16),
                pltpu.VMEM((8, M, 128), F32),
                pltpu.VMEM((2, 8, M, 128), BF16),
                pltpu.VMEM((G, M, DH), BF16),
                pltpu.SMEM((1,), jnp.int32),
                pltpu.SemaphoreType.DMA((6, NS)),
                pltpu.SemaphoreType.DMA((2,)),
            ],
            compiler_params=pltpu.CompilerParams(vmem_limit_bytes=120 * 1024 * 1024, disable_bounds_checks=True, disable_semaphore_checks=True,
                                                 flags=({flags: True} if flags else None)),
        )(A_x.reshape(M, D), A_k_cache, A_v_cache, A_wq, A_wo,
          B_x.reshape(4, BM, D), B_k_cache, B_v_cache, B_wq, B_wo)
        return out.reshape(B, SQ, 2 * D)
    return fn


_IMPL = build(sa=4)


@jax.jit
def pallas_concat_heads__mha_block_cached__mha_block_cached__near_ridge_kernel(
        A_x, A_k_cache, A_v_cache, A_wq, A_wo, B_x, B_k_cache, B_v_cache, B_wq, B_wo):
    return _IMPL(A_x, A_k_cache, A_v_cache, A_wq, A_wo, B_x, B_k_cache, B_v_cache, B_wq, B_wo)
```

```python
from typing import NamedTuple

import jax
import jax.numpy as jnp
from jax import lax
import jax.experimental.pallas as pl
import jax.experimental.pallas.tpu as pltpu

B, SQ, D = 16, 32, 1024
H, SK, DH = 32, 32, 128
M = B * SQ
LANES = 128
GB = LANES // SK
G = 8
NG = H // G
NS = 2 * NG
BM, BK = M // 4, D // 4
XROWS = 16
SCORE_SCALE_LOG2 = DH ** -0.5 * 1.4426950408889634
F32, BF16 = jnp.float32, jnp.bfloat16

LHS = (
    ((1, 0, 0), (1, 1, 1)), ((1, 1, 0), (1, 1, 1)), ((1, 0, 0), (1, 0, 1)), ((1, 1, 1),),
    ((1, 0, 1), (-1, 1, 1)), ((1, 0, 0),), ((1, 1, 0), (-1, 0, 0)),
)
RHS = (
    ((1, 0, 0), (1, 1, 1)), ((1, 0, 0),), ((1, 1, 1),), ((1, 1, 0), (-1, 0, 0)),
    ((1, 1, 0), (1, 1, 1)), ((1, 0, 1), (-1, 1, 1)), ((1, 0, 0), (1, 0, 1)),
)
OUT = (
    ((0, 0), ((1, 0), (-1, 2), (1, 3), (1, 4))),
    ((0, 1), ((1, 2), (1, 5))),
    ((1, 0), ((1, 1), (1, 3))),
    ((1, 1), ((1, 0), (-1, 1), (1, 5), (1, 6))),
)
FLIP = (0, 1, 1, 0, 1, 0, 1)
ROUNDS = (
    ((1, 0), (1, 1)), ((2, 0), (2, 1)), ((3, 0), (4, 0)), ((3, 1), (4, 1)),
    ((0, 0), (0, 1)), ((5, 0), (6, 0)), ((5, 1), (6, 1)),
)


class Plan(NamedTuple):
    order: str
    q_outer: str
    q_rounds: str
    o_outer: str
    o_rounds: str
    quadrants: str


START = "x10 x11 q00 m17 x00 b22 b33 m03 b32 r2 b23 r2 x01 m27 q10 m37 m47 q01 m57 m67"
START_ROUNDS = "0125436 4102356 0125463 5014263 1524036 0125436 1564023"
FIRST = Plan(
    "Wq11 Q7 Wq00 Q14 Wq01 Q7 Wq10 Q21",
    "2015364", "0425136 5021436 0615342 0425136 0125436 0425136 0125364",
    "", "", "")
SECOND = Plan(
    "Wk K0 K1 K2 K3 Wv V0 V1 V2 K6 K4 K5 V3 Wo00 Wo11 O1 V4 O1 K7 O1 V5 V6 O5 V7 O6 Wo10 O21 "
    "Wo01 O14",
    "", "",
    "0134256", "1034652 0316452 0164253 0124536 0152436 0124536 0124635", "3021")
EARLY = Plan(
    "Wq Q7 Wk K0 Q2 K1 K2 Q1 K3 Q1 K4 K5 Q2 K6 Q2 K7 Q1 Wv V0 Q1 V2 V1 Q1 V3 Q1 V4 Q2 V5 V6 "
    "Q1 V7 Q27 Wo O5 Wx X2 O1 X3 O1 X3 O1 X3 O1 X3 O1 X3 O1 X3 O1 X3 O1 X3 O1 X3 O1 X3 O1 X3 "
    "O1 X3 O1 X3 O1 X3 O1 X3 O1 X3 O1 X3 O1 X3 O26",
    "1502643", "0125436 0126453 0152436 0125436 0125436 0152436 0126435",
    "0432165", "0125436 0125436 1025436 0125436 0125463 1524063 0125463", "3021")
LATE = Plan(
    "Wq Q1 Wk K0 K1 Q2 Wv V0 Q1 K2 Q1 V1 Q2 V2 Q1 K3 K4 Q1 V3 Q2 K5 Q1 V4 Q1 K6 Q1 V5 Q1 K7 "
    "Q1 V6 Q1 V7 Q32 Wo O49",
    "2051364", "0152436 3125406 0125436 0126543 0124536 0125436 0125436",
    "0423165", "0125436 0162543 0125436 0124536 0124635 0125436 0125436", "3021")
LAST = Plan(
    "Wk K0 K1 K2 K3 Wv V0 V1 V2 K6 K4 K5 V3 Wo O1 V4 O1 K7 O1 V5 V6 O3 V7 O43",
    "", "",
    "0143256", "1034652 1034652 6014253 0142356 0416532 0124635 0124635", "3021")


def _term(spec, x):
    val = x(*spec[0][1:])
    for sign, *idx in spec[1:]:
        val = val + x(*idx) if sign > 0 else val - x(*idx)
    return val


def _outer_term(spec, blk, r, c):
    return _term(spec, lambda i, j: blk(2 * i + r, 2 * j + c))


class _Combiner:
    def __init__(self):
        self.products, self.done = {}, []

    def add(self, i, val):
        self.products[i] = val

    def ready(self):
        arrival = list(self.products)
        for rc, spec in OUT:
            if rc not in self.done and all(i in self.products for _, i in spec):
                self.done.append(rc)
                spec = sorted(spec, key=lambda t: arrival.index(t[1]))
                if spec[0][0] < 0:
                    spec[0], spec[1] = spec[1], spec[0]
                yield rc, _term(spec, lambda i: self.products[i])


def _kernel(ax, ak, av, awq, awo, bx, bk, bv, bwq, bwo, out_hbm,
            x_buf, xb_buf, xs_buf, wq_buf, k_buf, v_buf, wo_buf, q_first, q_buf, acc, out_buf,
            fence_ref, in_sems, out_sems):
    wq_hbm, k_hbm, v_hbm, wo_hbm = (awq, bwq), (ak, bk), (av, bv), (awo, bwo)

    def x_copy(r, c):
        idx = (pl.ds(r * M // 2, M // 2), pl.ds(c * D // 2, D // 2))
        return pltpu.make_async_copy(ax.at[idx], x_buf.at[idx], in_sems.at[4, 2 * r + c])

    def xb_copy(half):
        rows = pl.ds(half * (BM // 2), BM // 2)
        return pltpu.make_async_copy(bx.at[:, rows], xb_buf.at[:, rows], in_sems.at[4, 4 + half])

    buffers = {"q": wq_buf, "k": k_buf, "v": v_buf, "o": wo_buf}

    def whole_copy(kind, s):
        br, g = divmod(s, NG)
        src = {"q": lambda: wq_hbm[br].at[:, pl.ds(g * G * DH, G * DH)],
               "k": lambda: k_hbm[br].at[:, pl.ds(g * G, G)],
               "v": lambda: v_hbm[br].at[:, pl.ds(g * G, G)],
               "o": lambda: wo_hbm[br].at[pl.ds(g * G * DH, G * DH), :]}[kind]()
        return pltpu.make_async_copy(src, buffers[kind].at[s], in_sems.at["qkvo".index(kind), s])

    def wait_whole(kind, s):
        dst = buffers[kind].at[s]
        pltpu.make_async_copy(dst, dst, in_sems.at["qkvo".index(kind), s]).wait()

    def quadrant_copy(kind, s, r, c):
        rows, cols = r * D // 2, c * D // 2
        if kind == "q":
            src = awq.at[pl.ds(rows, D // 2), pl.ds(s * G * DH + cols, D // 2)]
        else:
            src = awo.at[pl.ds(s * G * DH + rows, D // 2), pl.ds(cols, D // 2)]
        return pltpu.make_async_copy(src, buffers[kind].at[s, pl.ds(rows, D // 2), pl.ds(cols, D // 2)],
                                     in_sems.at[5 + "qo".index(kind), 4 * s + 2 * r + c])

    def block_copy(r, c):
        idx = (pl.ds(r * BK, BK), pl.ds(c * BK, BK))
        return pltpu.make_async_copy(awq.at[idx], wq_buf.at[(0,) + idx], in_sems.at[7 + r // 2, r % 2 * 4 + c])

    def start_copy(tok):
        r, c = int(tok[1]), int(tok[2])
        return {"x": x_copy, "b": block_copy, "q": lambda r, c: quadrant_copy("q", 0, r, c)}[tok[0]](r, c)

    def first_quadrants(kind):
        tokens = FIRST.order.split() + SECOND.order.split()
        return [(int(tok[2]), int(tok[3])) for tok in tokens if tok[:2] == "W" + kind]

    for tok in START.split():
        if tok[0] in "xqb":
            start_copy(tok).start()
    for r, c in first_quadrants("q"):
        quadrant_copy("q", 1, r, c).start()
    for s in range(NS):
        if 1 <= s < NS - 1:
            whole_copy("q", s + 1).start()
        whole_copy("k", s).start()
        whole_copy("v", s).start()
        if s == 0:
            for r, c in first_quadrants("o"):
                quadrant_copy("o", 0, r, c).start()
        else:
            whole_copy("o", s).start()
        if s in (1, 2):
            xb_copy(s - 1).start()

    def wait_here(step, wait):
        pl.when(step > 0)(wait)

    def lhs_terms(quadrant):
        return [_term(spec, lambda r, c: quadrant[r, c]) for spec in LHS]

    def lhs_quadrants(blk, i1):
        return {(r, c): _outer_term(LHS[i1], blk, r, c) for r in range(2) for c in range(2)}

    def inner_products(lhs, weights, i1, rounds):
        shared = {}

        def rhs_block(j):
            local = {}

            def blk(r, c):
                return weights(r, c, slice(c * BK + j * LANES, c * BK + (j + 1) * LANES)).astype(F32)

            def get(r, c):
                cache = shared if (r == c and len(RHS[i1]) > 1) else local
                if (r, c, j) not in cache:
                    cache[r, c, j] = _outer_term(RHS[i1], blk, r, c ^ FLIP[i1])
                return cache[r, c, j]
            return get

        for n in rounds:
            fence_ref[0] = 0
            blocks = {j: rhs_block(j) for _, j in ROUNDS[int(n)]}
            yield [(i2, j, jnp.dot(lhs(i2), _term(RHS[i2], blocks[j]).astype(BF16),
                                   preferred_element_type=F32))
                   for i2, j in ROUNDS[int(n)]]

    def block_product(lhs_of, weights, emit, outer_order, rounds):
        outer = {(r, c, j): _Combiner() for r in range(2) for c in range(2) for j in range(2)}
        for i1, order in zip(map(int, outer_order), rounds.split()):
            inner = (_Combiner(), _Combiner())
            for results in inner_products(lhs_of(i1), weights, i1, order):
                for i2, j, val in results:
                    inner[j].add(i2, val)
                for j in range(2):
                    for (r, c), val in inner[j].ready():
                        c ^= FLIP[i1]
                        outer[r, c, j].add(i1, val)
                        for (rr, cc), res in outer[r, c, j].ready():
                            emit(2 * rr + r, 2 * (2 * cc + c) + j, res)
                yield results[0][2]

    def build_x_terms(i1):
        for j in range(2):
            def blk(r, c):
                cols = slice(c * BK + j * LANES, c * BK + (j + 1) * LANES)
                return x_buf[r * BM:(r + 1) * BM, cols].astype(F32)
            for i2, val in enumerate(lhs_terms(lhs_quadrants(blk, i1))):
                xs_buf[0, 7 * i1 + i2, j] = val.astype(BF16)

    def build_xb_strip(step, half, n, anchor):
        strips = BM // 2 // XROWS
        i1, rest = divmod(n, 2 * strips)
        j, k = divmod(rest, strips)
        rows = pl.ds(pl.multiple_of(half * (BM // 2) + k * XROWS, XROWS), XROWS)

        def blk(r, c):
            cols = slice(c * BK + j * LANES, c * BK + (j + 1) * LANES)
            return xb_buf[r, rows, cols].astype(F32)
        quadrant = lhs_quadrants(blk, i1)
        for d in range(2):
            quadrant[d, d] = jnp.where(step > 0, quadrant[d, d], anchor[k * XROWS:(k + 1) * XROWS])
        for i2, val in enumerate(lhs_terms(quadrant)):
            xs_buf[1, 7 * i1 + i2, j, rows] = val.astype(BF16)

    def x_terms(br, i1):
        return lambda i2: jnp.concatenate(
            [xs_buf[br, 7 * i1 + i2, j] for j in range(2)], axis=1)

    def weight_blocks(kind, s, arrived):
        def load(r, c, cols):
            assert any(w in arrived for w in (kind, f"{kind}{r // 2}{c // 2}", f"b{r}{c}"))
            return buffers[kind][s, r * BK:(r + 1) * BK, cols]
        return load

    def query_store(ref):
        def store(gb, h, val):
            ref[h, gb * BM:(gb + 1) * BM] = val.astype(BF16)
        return store

    def query_load(ref):
        return lambda gb, h: ref[h, gb * BM:(gb + 1) * BM]

    def attention_tiles(plan, n):
        quadrant, j = divmod(n, 2)
        rr, cc = divmod(int(plan.quadrants[quadrant]), 2)
        return [(2 * rr + r, 2 * (2 * cc + c) + j) for r in range(2) for c in range(2)]

    def probabilities(s, gb, h, q):
        k = k_buf[s, gb * GB:(gb + 1) * GB, h].reshape(GB * SK, DH)
        scores = lax.dot_general(k, q, (((1,), (1,)), ((), ())), preferred_element_type=F32)
        batch = lax.broadcasted_iota(jnp.int32, (SK, LANES), 1) // SQ
        own = scores[(GB - 1) * SK:]
        for b in reversed(range(GB - 1)):
            own = jnp.where(batch == b, scores[b * SK:(b + 1) * SK], own)
        e = jnp.exp2((own - jnp.max(own, axis=0, keepdims=True)) * SCORE_SCALE_LOG2)
        p = e * (1.0 / jnp.sum(e, axis=0, keepdims=True))
        return jnp.concatenate([jnp.where(batch == b, p, 0.0) for b in range(GB)], axis=0).astype(BF16)

    def weighted_values(s, gb, h, p):
        v = v_buf[s, gb * GB:(gb + 1) * GB, h].reshape(GB * SK, DH)
        return lax.dot_general(p, v, (((0,), (0,)), ((), ())), preferred_element_type=F32)

    def stage(step, s, plan, br, queries_in, queries_out, emit_out, x_half=None):
        probs, heads, arrived, stored = {}, {}, [], []

        def emit_queries(gb, h, val):
            stored.append((gb, h))
            queries_out(gb, h, val)

        def out_terms(i1):
            halves = [lhs_terms(lhs_quadrants(lambda r, c: heads[r, 2 * c + j], i1)) for j in range(2)]
            terms = [jnp.concatenate(pair, axis=1).astype(BF16) for pair in zip(*halves)]
            return lambda i2: terms[i2]

        queries = block_product(lambda i1: x_terms(br, i1), weight_blocks("q", s, arrived),
                                emit_queries, plan.q_outer, plan.q_rounds)
        outputs = block_product(out_terms, weight_blocks("o", s - 1, arrived),
                                emit_out, plan.o_outer, plan.o_rounds)
        strip = 0
        for tok in plan.order.split():
            kind, arg = tok[0], tok[1:]
            if kind == "Q":
                for _ in range(int(arg)):
                    next(queries)
            elif kind == "O":
                for _ in range(int(arg)):
                    anchor = next(outputs)
            elif kind == "K":
                assert "k" in arrived
                for gb, h in attention_tiles(plan, int(arg)):
                    assert (gb, h) not in stored
                    probs[gb, h] = probabilities(s - 1, gb, h, queries_in(gb, h))
            elif kind == "V":
                assert "v" in arrived
                for gb, h in attention_tiles(plan, int(arg)):
                    heads[gb, h] = weighted_values(s - 1, gb, h, probs.pop((gb, h)))
            elif kind == "X":
                assert "x" in arrived
                for _ in range(int(arg)):
                    build_xb_strip(step, x_half, strip, anchor)
                    strip += 1
            else:
                arrived.append(arg)
                at = s if arg[0] == "q" else s - 1
                if arg == "x":
                    pl.when(step < NG)(lambda: xb_copy(step - 2).wait())
                elif len(arg) == 1:
                    wait_here(step, lambda: wait_whole(arg, at))
                else:
                    wait_here(step, quadrant_copy(arg[0], at, int(arg[1]), int(arg[2])).wait)
        assert next(queries, None) is None and next(outputs, None) is None
        assert strip == (0 if x_half is None else 7 * BM // XROWS)

    def rows_of(r):
        return slice(r * BM, (r + 1) * BM)

    def first(step):
        arrived = []

        def built_x_terms(i1):
            assert all(f"x{r}{c}" in arrived for _, r, c in LHS[i1])
            build_x_terms(i1)
            return x_terms(0, i1)

        order = [tok[1] for tok in START.split() if tok[0] == "m"]
        queries = block_product(built_x_terms, weight_blocks("q", 0, arrived),
                                query_store(q_first), order, START_ROUNDS)
        for tok in START.split():
            if tok[0] in "mr":
                for _ in range(int(tok[-1])):
                    next(queries)
            else:
                wait_here(step, start_copy(tok).wait)
                arrived.append(tok)
        assert next(queries, None) is None

        stage(step, 1, FIRST, 0, None, query_store(q_buf), None)

    def second(step):
        def emit(r, n, val):
            acc[n, rows_of(r)] = val
        stage(step, 1, SECOND, 0, query_load(q_first), None, emit)

    def early(s):
        def emit(r, n, val):
            acc[n, rows_of(r)] = val + acc[n, rows_of(r)]
        stage(s, s, EARLY, 0, query_load(q_buf), query_store(q_buf), emit, x_half=s % 2)

    def late(s):
        def emit(r, n, val):
            val = val + acc[n, rows_of(r)]
            out_buf[(s - 1) // NG, n, rows_of(r)] = val.astype(BF16)
            acc[n, rows_of(r)] = jnp.where(s == NG, 0.0, val)
        stage(s, s, LATE, 1, query_load(q_buf), query_store(q_buf), emit)

    def last(step):
        for n in range(D // LANES):
            pltpu.make_async_copy(out_buf.at[0, n], out_hbm.at[:, pl.ds(n * LANES, LANES)],
                                  out_sems.at[0]).start()

        def emit(r, n, val):
            out_buf[1, n, rows_of(r)] = (val + acc[n, rows_of(r)]).astype(BF16)
            rows = pl.ds(r * BM, BM)
            pltpu.make_async_copy(out_buf.at[1, n, rows], out_hbm.at[rows, pl.ds(D + n * LANES, LANES)],
                                  out_sems.at[1]).start()
        stage(step, NS, LAST, 1, query_load(q_buf), None, emit)

    def run(step, _):
        pl.when(step == 1)(lambda: first(step))
        pl.when(step < 2)(lambda: second(step))
        pl.when(jnp.logical_and(step > 1, step < NG))(lambda: early(step))
        pl.when(jnp.logical_and(step >= NG, step < NS))(lambda: late(step))
        pl.when(step == NS)(lambda: last(step))
        return 0

    lax.fori_loop(1, NS + 1, run, 0)
    for br in (1, 0):
        pltpu.make_async_copy(out_buf.at[br], out_buf.at[br], out_sems.at[br]).wait()


@jax.jit
def pallas_concat_heads__mha_block_cached__mha_block_cached__near_ridge_kernel(
    A_x: jax.Array,
    A_k_cache: jax.Array,
    A_v_cache: jax.Array,
    A_wq: jax.Array,
    A_wo: jax.Array,
    B_x: jax.Array,
    B_k_cache: jax.Array,
    B_v_cache: jax.Array,
    B_wq: jax.Array,
    B_wo: jax.Array,
):
    out = pl.pallas_call(
        _kernel,
        out_shape=jax.ShapeDtypeStruct((M, 2 * D), BF16),
        in_specs=[pl.BlockSpec(memory_space=pl.ANY)] * 10,
        out_specs=pl.BlockSpec(memory_space=pl.ANY),
        scratch_shapes=[
            pltpu.VMEM((M, D), BF16),
            pltpu.VMEM((4, BM, D), BF16),
            pltpu.VMEM((2, 49, 2, BM, LANES), BF16),
            pltpu.VMEM((NS, D, G * DH), BF16),
            pltpu.VMEM((NS, B, G, SK, DH), BF16),
            pltpu.VMEM((NS, B, G, SK, DH), BF16),
            pltpu.VMEM((NS, G * DH, D), BF16),
            pltpu.VMEM((G, M, DH), BF16),
            pltpu.VMEM((G, M, DH), BF16),
            pltpu.VMEM((D // LANES, M, LANES), F32),
            pltpu.VMEM((2, D // LANES, M, LANES), BF16),
            pltpu.SMEM((1,), jnp.int32),
            pltpu.SemaphoreType.DMA((9, NS)),
            pltpu.SemaphoreType.DMA((2,)),
        ],
        compiler_params=pltpu.CompilerParams(
            vmem_limit_bytes=120 * 1024 * 1024,
            disable_semaphore_checks=True,
            flags={"XLA_TPU_RESCHEDULE_DMA_DONES": True},
        ),
    )(A_x.reshape(M, D), A_k_cache, A_v_cache, A_wq, A_wo,
      B_x.reshape(4, BM, D), B_k_cache, B_v_cache, B_wq, B_wo)
    return out.reshape(B, SQ, 2 * D)
```
